```python
import jax
import jax.numpy as jnp

def _softmax(x, axis=-1):
    return jax.nn.softmax(x, axis=axis)
def _gelu(x):
    return jax.nn.gelu(x, approximate=True)
def _silu(x):
    return jax.nn.silu(x)
def _sigmoid(x):
    return jax.nn.sigmoid(x)
def _layernorm(x, axis=-1, eps=1e-5):
    m = jnp.mean(x, axis=axis, keepdims=True)
    v = jnp.var(x, axis=axis, keepdims=True)
    return (x - m) / jnp.sqrt(v + eps)
def _scatter_add(tgt, idx, src, axis=0):
    return tgt.at[idx].add(src)
def _segment_sum(src, seg, n):
    return jax.ops.segment_sum(src, seg, n)
class _Rng:
    def __init__(self, key):
        self._k = key
    def _next(self):
        self._k, sub = jax.random.split(self._k)
        return sub
    def normal(self, shape):
        return jax.random.normal(self._next(), shape, dtype=jnp.bfloat16)
    def randint(self, lo, hi, shape):
        return jax.random.randint(self._next(), shape, lo, hi, dtype=jnp.int32)
    def uniform(self, shape, lo=0.0, hi=1.0):
        return jax.random.uniform(self._next(), shape, jnp.bfloat16, lo, hi)
    def permutation(self, n):
        return jax.random.permutation(self._next(), n)


kernel_name = 'standalone__depthwise_separable__vision'

def setup_inputs():
    _rng = _Rng(jax.random.key(int.from_bytes(__import__("os").urandom(4), "little")))
    _w = (lambda a: (lambda t: t.astype(jnp.bfloat16) if jnp.issubdtype(t.dtype, jnp.floating) else t)(jnp.asarray(a)))
    H = W = 384
    C = 384
    k = 1
    return {
        "x": _w((lambda *s: _rng.normal(s) * 0.05)(1, H, W, C)),
        "dw": _w((lambda *s: _rng.normal(s) * 0.05)(k, k, C)),
        "pw": _w((lambda *s: _rng.normal(s) * 0.05)(C, C)),
    }

def reference(x, dw, pw):
    B, H, W, C = x.shape
    k = dw.shape[0]
    pad = k // 2
    xp = jnp.pad(x, ((0,0),(pad,pad),(pad,pad),(0,0)))
    out = jnp.zeros_like(x)
    for i in range(k):
        for j in range(k):
            out = out + xp[:, i:i+H, j:j+W, :] * dw[i, j][None, None, None, :]
    return jnp.einsum('bhwc,cd->bhwd', out, pw)
```

```python
import jax
import jax.numpy as jnp
import jax.experimental.pallas as pl
import jax.experimental.pallas.tpu as pltpu

_S = 8
_R = 768
_TM = 48
_G1 = 13
_K = 4
_D0 = 16


@jax.jit
def pallas_standalone__depthwise_separable__vision_kernel(
    x: jax.Array,
    dw: jax.Array,
    pw: jax.Array,
):
    B, H, W, C = x.shape
    assert dw.shape == (1, 1, C) and pw.shape == (C, C)
    M = B * H * W
    G = M // (_S * _R)
    assert G * _S * _R == M
    nw = _R // _TM
    U2 = (G - _G1) * _S
    for u in range(U2):
        assert _D0 + _K * (u + 1) <= nw * (_G1 + u // _S)

    def kernel(x_hbm, dw_ref, pw_ref, o_hbm, buf, rsem, wsem):
        def rd(g):
            return pltpu.make_async_copy(x_hbm.at[g], buf.at[g], rsem.at[g])

        def wr(q):
            g = q // nw
            rows = pl.ds(pl.multiple_of((q % nw) * _TM, _TM), _TM)
            return pltpu.make_async_copy(
                buf.at[g, :, rows], o_hbm.at[g, :, rows], wsem.at[g])

        def compute(g, s):
            d = dw_ref[...].astype(jnp.float32)
            y = (buf[g, s].astype(jnp.float32) * d).astype(buf.dtype)
            buf[g, s] = jnp.dot(
                y, pw_ref[...], preferred_element_type=jnp.float32
            ).astype(buf.dtype)

        @pl.loop(0, G)
        def _(g):
            rd(g).start()

        @pl.loop(0, _G1)
        def _(g):
            rd(g).wait()

            @pl.loop(0, _S)
            def _(s):
                compute(g, s)

        @pl.loop(_G1, G)
        def _(g):
            rd(g).wait()

        @pl.loop(0, _D0)
        def _(q):
            wr(q).start()

        @pl.loop(0, U2)
        def _(u):
            for i in range(_K):
                wr(_D0 + u * _K + i).start()
            compute(_G1 + u // _S, u % _S)

        @pl.loop(_D0 + _K * U2, G * nw)
        def _(q):
            wr(q).start()

        @pl.loop(0, G)
        def _(g):
            pltpu.make_async_copy(buf.at[g], o_hbm.at[g], wsem.at[g]).wait()

    out = pl.pallas_call(
        kernel,
        in_specs=[
            pl.BlockSpec(memory_space=pl.ANY),
            pl.BlockSpec(memory_space=pltpu.VMEM),
            pl.BlockSpec(memory_space=pltpu.VMEM),
        ],
        out_specs=pl.BlockSpec(memory_space=pl.ANY),
        out_shape=jax.ShapeDtypeStruct((G, _S, _R, C), x.dtype),
        scratch_shapes=[
            pltpu.VMEM((G, _S, _R, C), x.dtype),
            pltpu.SemaphoreType.DMA((G,)),
            pltpu.SemaphoreType.DMA((G,)),
        ],
        compiler_params=pltpu.CompilerParams(
            vmem_limit_bytes=120 * 1024 * 1024),
    )(x.reshape(G, _S, _R, C), dw.reshape(1, C), pw)
    return out.reshape(B, H, W, C)
```

```python
import jax
import jax.numpy as jnp
import jax.experimental.pallas as pl
import jax.experimental.pallas.tpu as pltpu

_STREAMS = 6
_HALVES = 2
_ROWS = 1024
_PIECE = 16
_READ_STREAMS = 3
_UNIT = 128

_READ_AHEAD = 14
_READS_PER_UNIT = 8
_READ_TAIL = 6
_WRITE_AHEAD = 28
_WRITES_PER_UNIT = 14


@jax.jit
def pallas_standalone__depthwise_separable__vision_kernel(
    x: jax.Array,
    dw: jax.Array,
    pw: jax.Array,
):
    B, H, W, C = x.shape
    assert dw.shape == (1, 1, C) and pw.shape == (C, C)
    groups, ragged = divmod(B * H * W, _STREAMS * _HALVES * _ROWS)
    assert ragged == 0
    view = (groups, _STREAMS, _HALVES, _ROWS, C)

    pieces = _ROWS // _PIECE
    n_reads = groups * pieces
    n_writes = groups * _HALVES * pieces
    units_per_half = _ROWS // _UNIT
    units_per_group = _HALVES * units_per_half
    n_units = groups * units_per_group

    first_reads = pieces + _READ_AHEAD
    tail_start = n_reads - _READ_TAIL
    read_units = (tail_start - first_reads) // _READS_PER_UNIT
    write_units = n_units - read_units
    groups_waited = pl.cdiv(read_units, units_per_group)
    assert groups_waited < groups
    for u in range(read_units):
        issued = first_reads + _READS_PER_UNIT * (u + 1)
        assert issued >= (u // units_per_group + 1) * pieces
    for u in range(write_units):
        issued = _WRITE_AHEAD + _WRITES_PER_UNIT * (u + 1)
        assert issued * _PIECE <= (read_units + u) * _UNIT

    def kernel(x_hbm, dw_hbm, pw_hbm, o_hbm,
               buf, dw_ref, pw_ref, read_sems, tail_sem, write_sem, w_sems):

        def rows(i, size):
            return pl.ds(pl.multiple_of(i * size, size), size)

        def read_copy(idx, sem):
            return pltpu.make_async_copy(x_hbm.at[idx], buf.at[idx], sem)

        def start_read(p, sem=None):
            g = p // pieces
            sem = read_sems.at[g] if sem is None else sem
            for s in range(0, _STREAMS, _READ_STREAMS):
                for h in range(_HALVES):
                    idx = (g, pl.ds(s, _READ_STREAMS), h,
                           rows(p % pieces, _PIECE))
                    read_copy(idx, sem).start(priority=h)

        def wait_group(g):
            read_copy(g, read_sems.at[g]).wait()

        def start_write(q):
            idx = (q // (_HALVES * pieces), slice(None),
                   (q // pieces) % _HALVES, rows(q % pieces, _PIECE))
            pltpu.make_async_copy(buf.at[idx], o_hbm.at[idx], write_sem).start()

        def compute(u):
            idx = (u // units_per_group, slice(None),
                   (u // units_per_half) % _HALVES,
                   rows(u % units_per_half, _UNIT), slice(None))
            xs = buf[idx].reshape(_STREAMS * _UNIT, C)
            y = xs.astype(jnp.float32) * dw_ref[...].astype(jnp.float32)
            out = jnp.dot(y.astype(buf.dtype), pw_ref[...],
                          preferred_element_type=jnp.float32)
            buf[idx] = out.astype(buf.dtype).reshape(_STREAMS, _UNIT, C)

        pw_copy = pltpu.make_async_copy(pw_hbm, pw_ref, w_sems.at[0])
        dw_copy = pltpu.make_async_copy(dw_hbm, dw_ref, w_sems.at[1])
        pw_copy.start()
        dw_copy.start(priority=1)
        pl.loop(0, first_reads)(start_read)
        pw_copy.wait()
        dw_copy.wait()

        @pl.loop(0, read_units)
        def _(u):
            for i in range(_READS_PER_UNIT):
                start_read(first_reads + u * _READS_PER_UNIT + i)

            @pl.when(u % units_per_group == 0)
            def _():
                wait_group(u // units_per_group)

            compute(u)

        pl.loop(first_reads + read_units * _READS_PER_UNIT, tail_start)(
            start_read)
        pl.loop(tail_start, n_reads)(lambda p: start_read(p, tail_sem))
        pl.loop(groups_waited, groups - 1)(wait_group)

        last = (groups - 1, slice(None), slice(None))
        split = _ROWS - _READ_TAIL * _PIECE
        read_copy((*last, pl.ds(0, split)), read_sems.at[groups - 1]).wait()
        pl.loop(0, _WRITE_AHEAD)(start_write)
        read_copy((*last, pl.ds(split, _ROWS - split)), tail_sem).wait()

        @pl.loop(0, write_units)
        def _(u):
            for i in range(_WRITES_PER_UNIT):
                start_write(_WRITE_AHEAD + u * _WRITES_PER_UNIT + i)
            compute(read_units + u)

        pl.loop(_WRITE_AHEAD + write_units * _WRITES_PER_UNIT, n_writes)(
            start_write)
        pltpu.make_async_copy(buf, o_hbm, write_sem).wait()

    out = pl.pallas_call(
        kernel,
        in_specs=[pl.BlockSpec(memory_space=pl.ANY)] * 3,
        out_specs=pl.BlockSpec(memory_space=pl.ANY),
        out_shape=jax.ShapeDtypeStruct(view, x.dtype),
        scratch_shapes=[
            pltpu.VMEM(view, x.dtype),
            pltpu.VMEM((1, C), dw.dtype),
            pltpu.VMEM((C, C), pw.dtype),
            pltpu.SemaphoreType.DMA((groups,)),
            pltpu.SemaphoreType.DMA(()),
            pltpu.SemaphoreType.DMA(()),
            pltpu.SemaphoreType.DMA((2,)),
        ],
        compiler_params=pltpu.CompilerParams(
            vmem_limit_bytes=120 * 1024 * 1024,
            disable_bounds_checks=True,
        ),
    )(x.reshape(view), dw.reshape(1, C), pw)
    return out.reshape(B, H, W, C)
```
